```python
import jax
import jax.numpy as jnp

def _softmax(x, axis=-1):
    return jax.nn.softmax(x, axis=axis)
def _gelu(x):
    return jax.nn.gelu(x, approximate=True)
def _silu(x):
    return jax.nn.silu(x)
def _sigmoid(x):
    return jax.nn.sigmoid(x)
def _layernorm(x, axis=-1, eps=1e-5):
    m = jnp.mean(x, axis=axis, keepdims=True)
    v = jnp.var(x, axis=axis, keepdims=True)
    return (x - m) / jnp.sqrt(v + eps)
def _scatter_add(tgt, idx, src, axis=0):
    return tgt.at[idx].add(src)
def _segment_sum(src, seg, n):
    return jax.ops.segment_sum(src, seg, n)
class _Rng:
    def __init__(self, key):
        self._k = key
    def _next(self):
        self._k, sub = jax.random.split(self._k)
        return sub
    def normal(self, shape):
        return jax.random.normal(self._next(), shape, dtype=jnp.bfloat16)
    def randint(self, lo, hi, shape):
        return jax.random.randint(self._next(), shape, lo, hi, dtype=jnp.int32)
    def uniform(self, shape, lo=0.0, hi=1.0):
        return jax.random.uniform(self._next(), shape, jnp.bfloat16, lo, hi)
    def permutation(self, n):
        return jax.random.permutation(self._next(), n)


kernel_name = 'standalone__dcn_v2_cross__recsys'

def setup_inputs():
    _rng = _Rng(jax.random.key(int.from_bytes(__import__("os").urandom(4), "little")))
    _w = (lambda a: (lambda t: t.astype(jnp.bfloat16) if jnp.issubdtype(t.dtype, jnp.floating) else t)(jnp.asarray(a)))
    B, F, D, L = 16384, 26, 128, 6
    Din = min(F * D, 1024)
    return {
        "x0": _w((lambda *s: _rng.normal(s) * 0.05)(B, Din)),
        "ws": _w((lambda *s: _rng.normal(s) * 0.05)(L, Din, Din)),
        "bs": _w((lambda *s: _rng.normal(s) * 0.05)(L, Din)),
    }

def reference(x0, ws, bs):
    x = x0
    for l in range(ws.shape[0]):
        x = x0 * (x @ ws[l] + bs[l]) + x
    return x
```

```python
import jax
import jax.numpy as jnp
from jax import lax
import jax.experimental.pallas as pl
import jax.experimental.pallas.tpu as pltpu

f32 = jnp.float32
bf16 = jnp.bfloat16
u32 = jnp.uint32

TM, P, sub, ahead, xlate = 768, 256, 256, 2, 4


@jax.jit
def pallas_standalone__dcn_v2_cross__recsys_kernel(x0, ws, bs):
    B, D = x0.shape
    L = ws.shape[0]
    n = (B - P) // TM
    assert n * TM + P == B and P <= TM
    def kern(x_hbm, w_hbm, b_ref, o_hbm, xbuf, obuf, w_ref, wp_ref, bf_ref, wsem, xsem, osem, psem):
        wcp = lambda l: pltpu.make_async_copy(w_hbm.at[l], w_ref.at[l], wsem.at[l])
        xcp = lambda it, slot: pltpu.make_async_copy(
            x_hbm.at[pl.ds(pl.multiple_of(P + it * TM, 16), TM)], xbuf.at[slot], xsem.at[slot])
        ocp = lambda it, slot, r0, nr: pltpu.make_async_copy(
            obuf.at[slot, pl.ds(r0, nr)], o_hbm.at[pl.ds(pl.multiple_of(P + it * TM + r0, 16), nr)], osem.at[slot])
        pin = pltpu.make_async_copy(x_hbm.at[pl.ds(0, P)], xbuf.at[1, pl.ds(0, P)], psem.at[0])
        pout = pltpu.make_async_copy(obuf.at[1, pl.ds(0, P)], o_hbm.at[pl.ds(0, P)], psem.at[1])
        pin.start(); wcp(0).start()
        bf_ref[...] = b_ref[...].astype(f32)
        pin.wait()
        obuf[1, pl.ds(0, P), :] = xbuf[1, pl.ds(0, P), :]
        wcp(0).wait()
        for j in range(1, 1 + ahead):
            wcp(j).start()
        def pstep(l, c):
            @pl.when(l > 0)
            def _():
                wcp(l).wait()
                @pl.when(l + ahead < L)
                def _():
                    wcp(jnp.minimum(l + ahead, L - 1)).start()
            @pl.when(l == xlate)
            def _():
                xcp(0, 0).start()
            w = w_ref[l]
            wp_ref[l] = pltpu.bitcast(w, u32)
            xb = obuf[1, pl.ds(0, P), :]
            y = jnp.dot(xb, w, preferred_element_type=f32)
            v = xbuf[1, pl.ds(0, P), :].astype(f32) * (y + bf_ref[pl.ds(l, 1), :]) + xb.astype(f32)
            obuf[1, pl.ds(0, P), :] = v.astype(bf16)
            return c
        lax.fori_loop(0, L, pstep, 0)
        pout.start()
        def step(it, c):
            slot = it % 2
            xcp(it, slot).wait()
            @pl.when(it + 1 < n)
            def _():
                xcp(jnp.minimum(it + 1, n - 1), 1 - slot).start()
            @pl.when(it == 1)
            def _():
                pout.wait()
            @pl.when(it >= 2)
            def _():
                ocp(jnp.maximum(it - 2, 0), slot, 0, TM).wait()
            for s in range(TM // sub):
                sl = pl.ds(s * sub, sub)
                xb = xbuf[slot, sl, :]
                for l in range(L):
                    y = jnp.dot(xb, pltpu.bitcast(wp_ref[l], bf16), preferred_element_type=f32)
                    v = xbuf[slot, sl, :].astype(f32) * (y + bf_ref[l:l+1, :]) + xb.astype(f32)
                    xb = v.astype(bf16)
                obuf[slot, sl, :] = xb
                ocp(it, slot, s * sub, sub).start()
            return c
        lax.fori_loop(0, n, step, 0)
        ocp(n - 2, (n - 2) % 2, 0, TM).wait()
        ocp(n - 1, (n - 1) % 2, 0, TM).wait()
    return pl.pallas_call(
        kern,
        in_specs=[pl.BlockSpec(memory_space=pl.ANY), pl.BlockSpec(memory_space=pl.ANY),
                  pl.BlockSpec(memory_space=pltpu.VMEM)],
        out_specs=pl.BlockSpec(memory_space=pl.ANY),
        out_shape=jax.ShapeDtypeStruct((B, D), x0.dtype),
        scratch_shapes=[pltpu.VMEM((2, TM, D), bf16), pltpu.VMEM((2, TM, D), bf16),
                        pltpu.VMEM((L, D, D), bf16), pltpu.VMEM((L, D // 2, D), u32),
                        pltpu.VMEM((L, D), f32), pltpu.SemaphoreType.DMA((L,)),
                        pltpu.SemaphoreType.DMA((2,)), pltpu.SemaphoreType.DMA((2,)), pltpu.SemaphoreType.DMA((2,))],
        compiler_params=pltpu.CompilerParams(vmem_limit_bytes=100*2**20),
    )(x0, ws, bs)
```
